```python
import os as _os
_os.environ.setdefault("JAX_PLATFORMS", "cpu")
import jax
import jax.numpy as jnp

def _softmax(x, axis=-1):
    return jax.nn.softmax(x, axis=axis)
def _gelu(x):
    return jax.nn.gelu(x, approximate=True)
def _silu(x):
    return jax.nn.silu(x)
def _sigmoid(x):
    return jax.nn.sigmoid(x)
def _layernorm(x, axis=-1, eps=1e-5):
    m = jnp.mean(x, axis=axis, keepdims=True)
    v = jnp.var(x, axis=axis, keepdims=True)
    return (x - m) / jnp.sqrt(v + eps)
def _scatter_add(tgt, idx, src, axis=0):
    return tgt.at[idx].add(src)
def _segment_sum(src, seg, n):
    return jax.ops.segment_sum(src, seg, n)
class _Rng:
    def __init__(self, key):
        self._k = key
    def _next(self):
        self._k, sub = jax.random.split(self._k)
        return sub
    def normal(self, shape):
        return jax.random.normal(self._next(), shape, dtype=jnp.bfloat16)
    def randint(self, lo, hi, shape):
        return jax.random.randint(self._next(), shape, lo, hi, dtype=jnp.int32)
    def uniform(self, shape, lo=0.0, hi=1.0):
        return jax.random.uniform(self._next(), shape, jnp.bfloat16, lo, hi)
    def permutation(self, n):
        return jax.random.permutation(self._next(), n)


kernel_name = 'parallel_sum__mha_block__swiglu_ffn__prompt'

def setup_inputs():
    _rng = _Rng(jax.random.key(int.from_bytes(__import__("os").urandom(4), "little")))
    _w = (lambda a: (lambda t: t.astype(jnp.bfloat16) if jnp.issubdtype(t.dtype, jnp.floating) else t)(jnp.asarray(a)))
    def _A_setup():
        B, S, D, H = 1, 2048, 640, 32
        return {
            "x": _w((lambda *s: _rng.normal(s) * 0.05)(B, S, D)),
            "wqkv": _w((lambda *s: _rng.normal(s) * 0.1)(D, 3 * D)),
            "wo": _w((lambda *s: _rng.normal(s) * 0.05)(D, D)),
        }
    _A_in = _A_setup()

    def _B_setup():
        B, S, D, F = 1, 2048, 640, 1536
        return {
            "x": _w((lambda *s: _rng.normal(s) * 0.05)(B, S, D)),
            "w_gate": _w((lambda *s: _rng.normal(s) * 0.05)(D, F)),
            "w_up": _w((lambda *s: _rng.normal(s) * 0.05)(D, F)),
            "w_down": _w((lambda *s: _rng.normal(s) * 0.05)(F, D)),
        }
    _B_in = _B_setup()

    return {
        "A_x": _A_in["x"],
        "A_wqkv": _A_in["wqkv"],
        "A_wo": _A_in["wo"],
        "B_x": _B_in["x"],
        "B_w_gate": _B_in["w_gate"],
        "B_w_up": _B_in["w_up"],
        "B_w_down": _B_in["w_down"],
    }

def reference(A_x, A_wqkv, A_wo, B_x, B_w_gate, B_w_up, B_w_down):
    def _A_ref(x, wqkv, wo):
        B, S, D = x.shape
        H = 32
        Dh = D // H
        qkv = (lambda x, *d: x.transpose(*d))((x @ wqkv).reshape(B, S, 3, H, Dh), 2, 0, 3, 1, 4)
        q, k, v = qkv[0], qkv[1], qkv[2]
        scores = jnp.einsum("bhqd,bhkd->bhqk", q, k) * (Dh ** -0.5)
        p = _softmax(scores, axis=-1)
        o = jnp.einsum("bhqk,bhkd->bhqd", p, v)
        return (lambda x, *d: x.transpose(*d))(o, 0, 2, 1, 3).reshape(B, S, D) @ wo

    def _B_ref(x, w_gate, w_up, w_down):
        g = _silu(x @ w_gate)
        u = x @ w_up
        return (g * u) @ w_down

    x = A_x
    xn = _layernorm(x, axis=-1)
    return x + _A_ref(xn, A_wqkv, A_wo) + _B_ref(xn, B_w_gate, B_w_up, B_w_down)
```

```python
import functools
import math

import jax
import jax.numpy as jnp
from jax import lax
import jax.experimental.pallas as pl
import jax.experimental.pallas.tpu as pltpu

_H = 32
_LN_EPS = 1e-5
_BF = jnp.bfloat16
_F32 = jnp.float32
_NT = (((1,), (1,)), ((), ()))


def _kernel(x_hbm, wqkv_hbm, wo_hbm, wg_hbm, wu_hbm, wd_hbm, out_hbm,
            x_v, wqkv_v, wo_v, wg_v, wu_v, wd_v,
            xn_v, wqvt_v, k_v, qt_v, vt_v, ot_v, s_v, out_v,
            x_sem, w_sem, o_sem, *, S, D, F, T1, W, C, U, T3, FC):
    Dh = D // _H
    NS = D // 128
    n1 = S // T1
    n3 = S // T3
    qscale = (Dh ** -0.5) * math.log2(math.e)

    def x_copy(i):
        rows = pl.ds(i * T1, T1)
        return pltpu.make_async_copy(x_hbm.at[rows], x_v.at[rows], x_sem.at[i])

    w_copies = [
        pltpu.make_async_copy(src, dst, w_sem.at[n])
        for n, (src, dst) in enumerate(
            [(wqkv_hbm, wqkv_v), (wo_hbm, wo_v), (wg_hbm, wg_v), (wu_hbm, wu_v), (wd_hbm, wd_v)])
    ]
    x_copy(0).start()
    w_copies[0].start()
    for i in range(1, n1):
        x_copy(i).start()
    for c in w_copies[1:]:
        c.start()

    def layernorm(src, dst):
        x = x_v[pl.ds(src, T1), :].astype(_F32)
        xc = x - jnp.mean(x, axis=-1, keepdims=True)
        var = jnp.mean(xc * xc, axis=-1, keepdims=True)
        xn_v[pl.ds(dst, T1), :] = (xc * lax.rsqrt(var + _LN_EPS)).astype(_BF)

    s_v[1] = jnp.zeros((S, W), _F32)
    ot_v[pl.ds(D, 40), :] = jnp.zeros((40, S), _F32)
    x_copy(0).wait()
    layernorm(0, 0)
    w_copies[0].wait()
    wqvt_v[pl.ds(0, D), :] = wqkv_v[:, pl.ds(0, D)].T
    wqvt_v[pl.ds(D, D), :] = wqkv_v[:, pl.ds(2 * D, D)].T

    def proj_step(i, carry):
        @pl.when(i + 1 < n1)
        def _():
            x_copy(i + 1).wait()

        r0 = pl.multiple_of(i * T1, T1)
        rows = pl.ds(r0, T1)
        xn = xn_v[rows, :]
        k = jnp.dot(xn, wqkv_v[:, pl.ds(D, D)], preferred_element_type=_F32).astype(_BF)
        lane = lax.broadcasted_iota(jnp.int32, (T1, 128), 1)
        for j in range(NS):
            k_v[j, rows, :] = k[:, j * 128:(j + 1) * 128]
        for j in range(NS - 1):
            k_v[NS + j, rows, :] = jnp.where(
                lane < 64, k[:, (j + 1) * 128:(j + 2) * 128], k[:, j * 128:(j + 1) * 128])
        qvt = lax.dot_general(wqvt_v[...], xn, _NT, preferred_element_type=_F32)
        qt = (qvt[:D] * qscale).astype(_BF)
        for j in range(NS):
            qt_v[j, :, rows] = qt[j * 128:(j + 1) * 128]
        for j in range(NS - 1):
            qt_v[NS + j, pl.ds(0, 64), rows] = qt[(j + 1) * 128:(j + 1) * 128 + 64]
            qt_v[NS + j, pl.ds(64, 64), rows] = qt[j * 128 + 64:(j + 1) * 128]
        vt_v[:, rows] = qvt[D:].astype(_BF).astype(_F32)
        nxt = jnp.minimum(i + 1, n1 - 1)
        layernorm(pl.multiple_of(nxt * T1, T1), pl.multiple_of((i + 1) * T1, T1))
        return carry

    lax.fori_loop(0, n1, proj_step, 0)

    NC = S // C
    n_items = (S // W) * _H

    def scores_setup(item):
        h = item % _H
        cols = pl.ds(pl.multiple_of((item // _H) * W, W), W)
        lo = h * Dh
        j = lo // 128
        slab = jnp.where((lo + Dh - 1) // 128 == j, j, NS + j)
        row = lax.broadcasted_iota(jnp.int32, (64, W), 0)
        keep = ((row - lo // 2) & 63) < Dh // 2
        q = pltpu.bitcast(qt_v[slab, :, cols], jnp.uint32)
        q = pltpu.bitcast(jnp.where(keep, q, jnp.uint32(0)), _BF)
        return slab, q

    def scores_chunk(slab, q, c, buf, mrun):
        keys = pl.ds(c * C, C)
        s = jnp.dot(k_v[slab, keys, :], q, preferred_element_type=_F32)
        s_v[buf, keys, :] = s
        mc = jnp.max(s.reshape(C // 8, 8, W), axis=0)
        return mc if mrun is None else jnp.maximum(mrun, mc)

    def pv_chunk(vrow, odd, c, buf, m, acc):
        keys = pl.ds(c * C, C)
        p = jnp.exp2(s_v[buf, keys, :] - m).astype(_BF)
        v = vt_v[pl.ds(vrow, 24), keys]
        row = lax.broadcasted_iota(jnp.int32, (24, C), 0)
        v = jnp.where(row == (0 if odd else Dh), 1.0, v)
        o = jnp.dot(v, p, preferred_element_type=_F32)
        return o if acc is None else acc + o

    def pv_store(item, odd, acc):
        valid = item >= 0
        it = jnp.maximum(item, 0)
        cols = pl.ds(pl.multiple_of((it // _H) * W, W), W)
        base = jnp.where(valid, ((it % _H) // 2) * (2 * Dh), D)
        if odd:
            o = acc * (1.0 / acc[0:1])
            r = pl.ds(pl.multiple_of(base + 16, 8), 8)
            row = lax.broadcasted_iota(jnp.int32, (8, W), 0)
            ot_v[r, cols] = jnp.where(row < 4, ot_v[r, cols], o[0:8])
            ot_v[pl.ds(pl.multiple_of(base + 24, 8), 16), cols] = o[8:24]
        else:
            ot_v[pl.ds(pl.multiple_of(base, 8), 24), cols] = acc * (1.0 / acc[Dh:Dh + 1])

    def v_row(item, odd):
        h = jnp.maximum(item, 0) % _H
        return pl.multiple_of((h // 2) * (2 * Dh) + (16 if odd else 0), 8)

    def attn_step(i, m):
        for u in range(U):
            item = i * U + u
            odd = (u + 1) % 2 == 1
            slab, q = scores_setup(item)
            vrow = v_row(item - 1, odd)
            mrun = acc = None
            for c in range(NC):
                mrun = scores_chunk(slab, q, c, u % 2, mrun)
                acc = pv_chunk(vrow, odd, c, (u + 1) % 2, m, acc)
            pv_store(item - 1, odd, acc)
            m = jnp.max(mrun, axis=0, keepdims=True)
        return m

    m = lax.fori_loop(0, n_items // U, attn_step, jnp.zeros((1, W), _F32))
    acc = None
    for c in range(NC):
        acc = pv_chunk(D - 24, True, c, 1, m, acc)
    pv_store(jnp.int32(n_items - 1), True, acc)

    for c in w_copies[1:]:
        c.wait()

    def out_copy(i):
        rows = pl.ds(i * T3, T3)
        return pltpu.make_async_copy(out_v.at[rows], out_hbm.at[rows], o_sem.at[i])

    def tail_step(i, carry):
        rows = pl.ds(pl.multiple_of(i * T3, T3), T3)
        xn = xn_v[rows, :]
        acc = x_v[rows, :].astype(_F32)
        hs = []
        for f in range(F // FC):
            fc = pl.ds(f * FC, FC)
            g = jnp.dot(xn, wg_v[:, fc], preferred_element_type=_F32)
            u = jnp.dot(xn, wu_v[:, fc], preferred_element_type=_F32)
            hs.append((g * jax.nn.sigmoid(g) * u).astype(_BF))
        o = ot_v[pl.ds(0, D), rows].T.astype(_BF)
        acc += jnp.dot(o, wo_v[...], preferred_element_type=_F32)
        for f in range(F // FC):
            acc += jnp.dot(hs[f], wd_v[pl.ds(f * FC, FC), :], preferred_element_type=_F32)
        out_v[rows, :] = acc.astype(_BF)
        out_copy(i).start()
        return carry

    lax.fori_loop(0, n3, tail_step, 0)
    for i in range(n3):
        out_copy(i).wait()


@jax.jit
def pallas_parallel_sum__mha_block__swiglu_ffn__prompt_kernel(
    A_x: jax.Array,
    A_wqkv: jax.Array,
    A_wo: jax.Array,
    B_x: jax.Array,
    B_w_gate: jax.Array,
    B_w_up: jax.Array,
    B_w_down: jax.Array,
):
    T1, W, C, U, T3, FC = 512, 512, 128, 8, 512, 512
    del B_x
    B, S, D = A_x.shape
    F = B_w_gate.shape[1]
    NS = D // 128
    kern = functools.partial(_kernel, S=S, D=D, F=F, T1=T1, W=W, C=C, U=U, T3=T3, FC=FC)
    any_spec = pl.BlockSpec(memory_space=pl.ANY)
    out = pl.pallas_call(
        kern,
        out_shape=jax.ShapeDtypeStruct((S, D), A_x.dtype),
        in_specs=[any_spec] * 6,
        out_specs=any_spec,
        scratch_shapes=[
            pltpu.VMEM((S, D), _BF),
            pltpu.VMEM((D, 3 * D), _BF),
            pltpu.VMEM((D, D), _BF),
            pltpu.VMEM((D, F), _BF),
            pltpu.VMEM((D, F), _BF),
            pltpu.VMEM((F, D), _BF),
            pltpu.VMEM((S + T1, D), _BF),
            pltpu.VMEM((2 * D, D), _BF),
            pltpu.VMEM((2 * NS - 1, S, 128), _BF),
            pltpu.VMEM((2 * NS - 1, 128, S), _BF),
            pltpu.VMEM((D, S), _F32),
            pltpu.VMEM((D + 40, S), _F32),
            pltpu.VMEM((2, S, W), _F32),
            pltpu.VMEM((S, D), _BF),
            pltpu.SemaphoreType.DMA((S // T1,)),
            pltpu.SemaphoreType.DMA((5,)),
            pltpu.SemaphoreType.DMA((S // T3,)),
        ],
        compiler_params=pltpu.CompilerParams(vmem_limit_bytes=100 * 2**20),
    )(A_x.reshape(S, D), A_wqkv, A_wo, B_w_gate, B_w_up, B_w_down)
    return out.reshape(B, S, D)
```

```python
import functools
import math

import jax
import jax.numpy as jnp
from jax import lax
import jax.experimental.pallas as pl
import jax.experimental.pallas.tpu as pltpu

_BF = jnp.bfloat16
_F32 = jnp.float32
_U32 = jnp.uint32

_H = 32
_LN_EPS = 1e-5
_X_ROWS = (0, 256, 768, 1664, 2048)
_TK = 128
_T = 512
_W = 256
_C = 256
_NV = 160
_LAG = 2
_UNROLL = 16
_PACED = 17


def _mm(a, b):
    return jnp.dot(a, b, preferred_element_type=_F32)


def _mm_nt(a, b):
    return lax.dot_general(a, b, (((1,), (1,)), ((), ())), preferred_element_type=_F32)


def _cat(parts, axis):
    return jnp.concatenate(list(parts), axis=axis)


def _blocks(c11, c12, c21, c22):
    return _cat([_cat([c11, c12], 1), _cat([c21, c22], 1)], 0)


def _quarters(a, rows, cols):
    return a[:rows, :cols], a[:rows, cols:2 * cols], a[rows:, :cols], a[rows:, cols:2 * cols]


def _strassen_lhs(a11, a12, a21, a22):
    return [a.astype(_BF) for a in
            (a11 + a22, a21 + a22, a11, a22, a11 + a12, a21 - a11, a12 - a22)]


def _strassen_rhs(b11, b12, b21, b22):
    f11, f12, f21, f22 = (b.astype(_F32) for b in (b11, b12, b21, b22))
    return [b.astype(_BF) for b in
            (f11 + f22, b11, f12 - f22, f21 - f11, b22, f11 + f12, f21 + f22)]


def _strassen_add(init, lhs, rhs_ref):
    order = (0, 1, 3, 4, 2, 6, 5)
    signs = ((1, 0, 0, 1, -1, 0, 1), (0, 0, 1, 0, 1, 0, 0),
             (0, 1, 0, 1, 0, 0, 0), (1, -1, 1, 0, 0, 1, 0))
    prods = {j: _mm(lhs[j], pltpu.bitcast(rhs_ref[j], _BF)) for j in order}
    out = []
    for c, sign in zip(init, signs):
        for j in order:
            if sign[j]:
                c = c + prods[j] if sign[j] > 0 else c - prods[j]
        out.append(c)
    return out


def _silu(g):
    half = 0.5 * g
    return half + half * jnp.tanh(half)


def _after(value, zero):
    return pltpu.bitcast(pltpu.bitcast(value, _U32) | zero, _BF)


def _kernel(x_hbm, wqkv_hbm, wo_hbm, wg_hbm, wu_hbm, wd_hbm, out_hbm,
            x_v, wo_v, wos_v, k_v, kb_v, qf_v, q_v, v_v, y_v, s_v, pos_s,
            x_sem, w_sem, o_sem):
    S, D = x_hbm.shape
    F = wg_hbm.shape[1]
    Dh = D // _H
    G = 8 * Dh
    n_items = S // _W * _H
    n_steps = S // _C
    s_sem = len(_X_ROWS) - 1

    def projections(wqkv_v, wt_v, wg_v, wu_v, wd_v, xn_v, kf_v, kp_v, wgs_v, wus_v, wds_v):
        def x_copy(i):
            rows = pl.ds(_X_ROWS[i], _X_ROWS[i + 1] - _X_ROWS[i])
            return pltpu.make_async_copy(x_hbm.at[rows], x_v.at[rows], x_sem.at[i])

        wq_copy, wk_copy, wv_copy = (
            pltpu.make_async_copy(wqkv_hbm.at[:, pl.ds(j * D, D)], wqkv_v.at[j], w_sem.at[j])
            for j in range(3))
        wg_copy, *late_copies = (
            pltpu.make_async_copy(src, dst, w_sem.at[3 + j]) for j, (src, dst) in
            enumerate([(wg_hbm, wg_v), (wu_hbm, wu_v), (wd_hbm, wd_v), (wo_hbm, wo_v)]))

        def layernorm(r0):
            zero = kp_v[pl.ds(pl.multiple_of(pos_s[1], 8), 8), :]
            x = _after(x_v[pl.ds(r0, _TK), :], _cat([zero] * (_TK // 16), 0)).astype(_F32)
            xc = x - jnp.mean(x, axis=-1, keepdims=True)
            var = jnp.mean(xc * xc, axis=-1, keepdims=True)
            xn_v[pl.ds(r0, _TK), :] = (xc * lax.rsqrt(var + _LN_EPS)).astype(_BF)

        def k_projection(r0):
            k = _mm(xn_v[pl.ds(r0, _TK), :], wqkv_v[1]).astype(_BF)
            if r0 < _NV:
                for g in range(_H // 8):
                    kf_v[g, pl.ds(r0, _TK), :] = k.astype(_F32)[:, G * g:G * (g + 1)]
            kp_v[pl.ds(r0 // 2, _TK // 2), :] = pltpu.bitcast(k, _U32)

        x_copy(0).start()
        wk_copy.start()
        for j, pos in enumerate((2 * S, S // 2, n_items, _H)):
            pos_s[j] = pos
        kp_v[pl.ds(S // 2, 8), :] = jnp.zeros((8, D), _U32)
        q_v[n_items, pl.ds(0, 8), pl.ds(0, 128)] = jnp.zeros((8, 128), _U32)
        v_v[_H, pl.ds(0, 8), pl.ds(0, 128)] = jnp.zeros((8, 128), _F32)
        s_v[pl.ds(S - _LAG * _C, S + _LAG * _C), :] = jnp.zeros((S + _LAG * _C, _W), _F32)
        x_copy(0).wait()
        x_copy(1).start()
        layernorm(0)
        wk_copy.wait()
        for r0 in range(0, S, _TK):
            if r0 + _TK in _X_ROWS[:-1]:
                j = _X_ROWS.index(r0 + _TK)
                x_copy(j).wait()
                if j + 1 < s_sem:
                    x_copy(j + 1).start()
                if j + 2 == s_sem:
                    for copy in (wq_copy, wv_copy, wg_copy):
                        copy.start()
                if j + 1 == s_sem:
                    wq_copy.wait()
                    wv_copy.wait()
                    for copy in late_copies:
                        copy.start()
                    wt_v[pl.ds(0, D), :] = wqkv_v[0].T
                    wt_v[pl.ds(D, D), :] = wqkv_v[2].T
            if r0 + _TK < S:
                layernorm(r0 + _TK)
            k_projection(r0)

        def weight_sums(half, weights, part, zero):
            tiles = [(w_v, ws_v, r, c) for w_v, ws_v in weights
                     for r in range(0, ws_v.shape[1], 16) for c in range(0, ws_v.shape[2], 128)]
            for w_v, ws_v, r, c in tiles[part * len(tiles) // 7:(part + 1) * len(tiles) // 7]:
                r = half * ws_v.shape[1] + r
                top = pl.ds(pl.multiple_of(r, 16), 16)
                bottom = pl.ds(pl.multiple_of(2 * ws_v.shape[1] + r, 16), 16)
                left, right = pl.ds(c, 128), pl.ds(ws_v.shape[2] + c, 128)
                for j, b in enumerate(_strassen_rhs(
                        _after(w_v[top, left], zero), w_v[top, right],
                        w_v[bottom, left], _after(w_v[bottom, right], zero))):
                    ws_v[j, pl.ds(pl.multiple_of(r // 2, 8), 8), left] = pltpu.bitcast(b, _U32)

        def qv_step(i, carry, weights):
            toks = pl.ds(pl.multiple_of(i * _T, _T), _T)
            xn = xn_v[toks, :]
            row = lax.broadcasted_iota(jnp.int32, (8, _T), 0)
            zero = jnp.zeros((8, _T), _U32)
            blocks = [(i * (_T // _W) + b, slice(b * _W, (b + 1) * _W)) for b in range(_T // _W)]
            for g in range(_H // 8):
                qt = _mm_nt(wt_v[pl.ds(g * G, G), :], xn)
                qt = (qt * (Dh ** -0.5 * math.log2(math.e))).astype(_BF)
                for b, cols in blocks:
                    qf_v[b * (_H // 8) + g] = qt[:, cols].astype(_F32)
                qt = pltpu.bitcast(qt, _U32)
                for u in range(8):
                    r0, lo = u * Dh // 2 // 8 * 8, u * Dh // 2 % 8
                    q = _cat([jnp.where(row >= lo, qt[r0:r0 + 8], zero),
                              jnp.where(row < lo + Dh // 2 - 8, qt[r0 + 8:r0 + 16], zero)], 0)
                    for b, cols in blocks:
                        q_v[b * _H + 8 * g + u] = q[:, cols]
                weight_sums(i & 1, weights, 2 * g, q_v[pos_s[2], pl.ds(0, 8), pl.ds(0, 128)])

                vt = _mm_nt(wt_v[pl.ds(D + g * G, G), :], xn).astype(_BF).astype(_F32)
                for u in range(8):
                    r0 = u * Dh // 8 * 8
                    if u % 2 == 0:
                        v = [vt[r0:r0 + 16], jnp.where(row == Dh - 16, 1.0, vt[r0 + 16:r0 + 24])]
                    else:
                        v = [jnp.where(row == 0, 1.0, vt[r0:r0 + 8]), vt[r0 + 8:r0 + 24]]
                    v_v[8 * g + u, :, toks] = _cat(v, 0)
                weight_sums(i & 1, weights, 2 * g + 1,
                            pltpu.bitcast(v_v[pos_s[3], pl.ds(0, 8), pl.ds(0, 128)], _U32))
            return carry

        wg_copy.wait()
        lax.fori_loop(0, 2, functools.partial(qv_step, weights=[(wg_v, wgs_v)]), 0)
        for copy in late_copies:
            copy.wait()
        lax.fori_loop(2, 4, functools.partial(
            qv_step, weights=[(wu_v, wus_v), (wd_v, wds_v), (wo_v, wos_v)]), 0)

        def ffn_step(i, carry):
            rows = pl.ds(pl.multiple_of(i * _T, _T), _T)
            xn = xn_v[rows, :]
            xs = _strassen_lhs(*_quarters(xn.astype(_F32), _T // 2, 256))

            def first_layer(w_v, ws_v):
                rest = _mm(xn[:, 512:], w_v[pl.ds(512, D - 512), :])
                return _strassen_add(_quarters(rest, _T // 2, F // 2), xs, ws_v)

            h = [_silu(g) * u for g, u in zip(first_layer(wg_v, wgs_v), first_layer(wu_v, wus_v))]
            x = x_v[rows, :].astype(_F32)
            y_v[rows, pl.ds(0, 512)] = _blocks(
                *_strassen_add(_quarters(x, _T // 2, 256), _strassen_lhs(*h), wds_v))
            y_v[rows, pl.ds(512, D - 512)] = x[:, 512:] + _mm(
                _blocks(*h).astype(_BF), wd_v[:, pl.ds(512, D - 512)])

            packed_rows = pl.ds(pl.multiple_of(i * (_T // 2), _T // 2), _T // 2)
            k = kp_v[packed_rows, :]
            k = _cat([k, k[:, :128]], 1)
            for pair in range(_H // 2):
                lo = pair * 2 * Dh // 16 * 16
                k_v[pair, packed_rows, :] = k[:, lo:lo + 128]
            for d in range(G):
                kb_v[i * 8 + d // Dh, :, pl.ds(d % Dh * 128, 128)] = jnp.broadcast_to(
                    kf_v[i, pl.ds(0, _NV), pl.ds(d, 1)], (_NV, 128))
            return carry

        lax.fori_loop(0, S // _T, ffn_step, 0)

    def attention(qb_v, o_v):
        n_mxu = (S - _NV) // 2
        bounds = [n_mxu // 16 * c // n_steps * 16 for c in range(n_steps + 1)]
        vpu_tiles = [(r0, t) for r0 in range(0, _NV, 8) for t in range(_W // 128)]

        def update_max(m, s, t0):
            m = list(m)
            for t in range(s.shape[1] // 128):
                part = jnp.max(s[:, t * 128:(t + 1) * 128].reshape(-1, 8, 128), axis=0)
                m[t0 + t] = part if m[t0 + t] is None else jnp.maximum(m[t0 + t], part)
            return m

        def repeat_q(item, u, features):
            for d in features:
                r0, r = divmod(u % 8 * Dh + d, 8)
                q = qf_v[(item & (n_items - 1)) >> 3, pl.ds(8 * r0, 8), :]
                q = jnp.broadcast_to(q[r:r + 1], (8, _W))
                qb_v[u % 2, d] = q
                if d == _PACED:
                    s_v[pl.ds(2 * S + u % 2 * 16, 8), :] = q

        def vpu_scores(pos, item, u, r0, t, m):
            lanes = pl.ds(t * 128, 128)
            sums = [None, None]
            for d in range(Dh):
                q = s_v[pl.ds(pos + u % 2 * 16, 8), lanes] if d == _PACED else qb_v[u % 2, d, :, lanes]
                term = kb_v[item & (_H - 1), pl.ds(r0, 8), pl.ds(d * 128, 128)] * q
                sums[d % 2] = term if sums[d % 2] is None else sums[d % 2] + term
            s = sums[0] + sums[1]
            s_v[pl.ds(u % 2 * S + r0, 8), lanes] = s
            return update_max(m, s, t)

        def scores(pos, item, u, c, m):
            above = u % 8 * Dh // 16 - u % 8 // 2 * 2 * Dh // 16
            zero = jnp.zeros((8, _W), _U32)
            q = pltpu.bitcast(_cat([zero] * above + [q_v[item]] + [zero] * (6 - above), 0), _BF)
            lo, hi = bounds[c], bounds[c + 1]
            halves = []
            for r0 in (_NV + lo, _NV + n_mxu + lo):
                k = k_v[(item & (_H - 1)) >> 1, pl.ds(r0 // 2, (hi - lo) // 2), :]
                halves.append((r0, _mm(pltpu.bitcast(k, _BF), q)))
            stops = [(e + 1) * n_mxu / len(vpu_tiles) - lo for e in range(len(vpu_tiles))]
            stops = [(round(at / 8) * 8, tile)
                     for at, tile in zip(stops, vpu_tiles) if 0 < at <= hi - lo]
            done = 0
            for upto, tile in stops + [(hi - lo, None)]:
                if upto > done:
                    for r0, s in halves:
                        s_v[pl.ds(u % 2 * S + r0 + done, upto - done), :] = s[done:upto]
                    done = upto
                if tile is not None:
                    m = vpu_scores(pos, item, u, *tile, m)
            for _, s in halves:
                m = update_max(m, s, 0)
            return m

        def weighted_values(item, u, c, m, acc):
            p = jnp.exp2(s_v[pl.ds(u % 2 * S + c * _C, _C), :] - m).astype(_BF)
            o = _mm(v_v[item & (_H - 1), :, pl.ds(c * _C, _C)], p)
            return o if c == 0 else acc + o

        def attention_step(i, carry):
            acc, m2, m1 = carry
            pos = pl.multiple_of(pos_s[0], 16)
            for u in range(_UNROLL):
                item = i * _UNROLL + u
                m = [None] * (_W // 128)
                for c in range(n_steps):
                    m = scores(pos, item, u, c, m)
                    if c < _LAG:
                        acc = weighted_values(item - 2, u - 2, n_steps - _LAG + c, m2, acc)
                    else:
                        acc = weighted_values(item - 1, u - 1, c - _LAG, m1, acc)
                    if c == _LAG - 1:
                        o_v[item] = acc
                    repeat_q(item + 1, u + 1, range(c * Dh // n_steps, (c + 1) * Dh // n_steps))
                m2, m1 = m1, jnp.max(_cat(m, 1), axis=0, keepdims=True)
            return acc, m2, m1

        repeat_q(0, 0, range(Dh))
        acc, m2, m1 = lax.fori_loop(
            0, n_items // _UNROLL, attention_step,
            (jnp.zeros((24, _W), _F32), jnp.zeros((1, _W), _F32), jnp.zeros((1, _W), _F32)))

        def out_copy(b):
            rows = pl.ds(b * _W, _W)
            return pltpu.make_async_copy(x_v.at[rows], out_hbm.at[rows], o_sem.at[b])

        def merged_heads(b, t):
            row = lax.broadcasted_iota(jnp.int32, (8, 128), 0)
            parts = []
            for h in range(0, _H, 2):
                even = o_v[b * _H + h + 2, :, pl.ds(t * 128, 128)]
                odd = o_v[b * _H + h + 3, :, pl.ds(t * 128, 128)]
                even = even * (1.0 / even[Dh:Dh + 1])
                odd = odd * (1.0 / odd[0:1])
                parts += [even[:16], jnp.where(row < Dh - 16, even[16:], odd[:8]), odd[8:]]
            return _cat(parts, 0).T

        for c in range(n_steps - _LAG, n_steps):
            acc = weighted_values(n_items - 2, 0, c, m2, acc)
        o_v[n_items] = acc
        for b in range(S // _W):
            rows = pl.ds(b * _W, _W)
            o = _cat([merged_heads(b, t) for t in range(_W // 128)], 0)
            y = y_v[rows, :]
            right = y[:, 512:] + _mm(o.astype(_BF), wo_v[:, pl.ds(512, D - 512)])
            left = y[:, :512] + _mm(
                o.astype(_BF)[:, 512:], wo_v[pl.ds(512, D - 512), pl.ds(0, 512)])
            left = _strassen_add(_quarters(left, _W // 2, 256),
                                 _strassen_lhs(*_quarters(o, _W // 2, 256)), wos_v)
            x_v[rows, :] = _cat([_blocks(*left), right], 1).astype(_BF)
            out_copy(b).start()
            for c in range(2 * b, min(n_steps, 2 * b + 2)):
                acc = weighted_values(n_items - 1, 1, c, m1, acc)
                if c == n_steps - 1:
                    o_v[n_items + 1] = acc
        for b in range(S // _W):
            out_copy(b).wait()

    pl.run_scoped(
        projections,
        pltpu.VMEM((3, D, D), _BF),
        pltpu.VMEM((2 * D, D), _BF),
        pltpu.VMEM((D, F), _BF),
        pltpu.VMEM((D, F), _BF),
        pltpu.VMEM((F, D), _BF),
        pltpu.VMEM((S, D), _BF),
        pltpu.VMEM((_H // 8, pl.cdiv(_NV, _TK) * _TK, G), _F32),
        pltpu.VMEM((S // 2 + 8, D), _U32),
        pltpu.VMEM((7, 128, F // 2), _U32),
        pltpu.VMEM((7, 128, F // 2), _U32),
        pltpu.VMEM((7, F // 4, 256), _U32))
    pl.run_scoped(
        attention,
        pltpu.VMEM((2, Dh, 8, _W), _F32),
        pltpu.VMEM((n_items + 2, 24, _W), _F32))


@jax.jit
def pallas_parallel_sum__mha_block__swiglu_ffn__prompt_kernel(
    A_x: jax.Array,
    A_wqkv: jax.Array,
    A_wo: jax.Array,
    B_x: jax.Array,
    B_w_gate: jax.Array,
    B_w_up: jax.Array,
    B_w_down: jax.Array,
):
    del B_x
    B, S, D = A_x.shape
    assert (B, S, D, B_w_gate.shape[1]) == (1, 2048, 640, 1536)
    Dh = D // _H
    n_items = S // _W * _H
    in_hbm = pl.BlockSpec(memory_space=pl.ANY)
    out = pl.pallas_call(
        _kernel,
        out_shape=jax.ShapeDtypeStruct((S, D), A_x.dtype),
        in_specs=[in_hbm] * 6,
        out_specs=in_hbm,
        scratch_shapes=[
            pltpu.VMEM((S, D), _BF),
            pltpu.VMEM((D, D), _BF),
            pltpu.VMEM((7, 128, 256), _U32),
            pltpu.VMEM((_H // 2, S // 2, 128), _U32),
            pltpu.VMEM((_H, _NV, Dh * 128), _F32),
            pltpu.VMEM((n_items // 8, 8 * Dh, _W), _F32),
            pltpu.VMEM((n_items + 1, 16, _W), _U32),
            pltpu.VMEM((_H + 1, 24, S), _F32),
            pltpu.VMEM((S, D), _F32),
            pltpu.VMEM((2 * S + 32, _W), _F32),
            pltpu.SMEM((4,), jnp.int32),
            pltpu.SemaphoreType.DMA((len(_X_ROWS) - 1,)),
            pltpu.SemaphoreType.DMA((7,)),
            pltpu.SemaphoreType.DMA((S // _W,)),
        ],
        compiler_params=pltpu.CompilerParams(vmem_limit_bytes=124 * 2**20),
    )(A_x.reshape(S, D), A_wqkv, A_wo, B_w_gate, B_w_up, B_w_down)
    return out.reshape(B, S, D)
```

```python
import functools
import math

import jax
import jax.numpy as jnp
from jax import lax
import jax.experimental.pallas as pl
import jax.experimental.pallas.tpu as pltpu

_BF = jnp.bfloat16
_F32 = jnp.float32
_U32 = jnp.uint32

_H = 32
_LN_EPS = 1e-5
_X_ROWS = (0, 256, 768, 1664, 2048)
_TK = 128
_T = 512
_W = 256
_C = 256
_NV = 160
_LAG = 2
_UNROLL = 16
_PACED = 17


def _mm(a, b):
    return jnp.dot(a, b, preferred_element_type=_F32)


def _mm_nt(a, b):
    return lax.dot_general(a, b, (((1,), (1,)), ((), ())), preferred_element_type=_F32)


def _cat(parts, axis):
    return jnp.concatenate(list(parts), axis=axis)


def _blocks(c11, c12, c21, c22):
    return _cat([_cat([c11, c12], 1), _cat([c21, c22], 1)], 0)


def _quarters(a, rows, cols):
    return a[:rows, :cols], a[:rows, cols:2 * cols], a[rows:, :cols], a[rows:, cols:2 * cols]


def _strassen_lhs(a11, a12, a21, a22):
    return [a.astype(_BF) for a in
            (a11 + a22, a21 + a22, a11, a22, a11 + a12, a21 - a11, a12 - a22)]


def _strassen_rhs(b11, b12, b21, b22):
    f11, f12, f21, f22 = (b.astype(_F32) for b in (b11, b12, b21, b22))
    return [b.astype(_BF) for b in
            (f11 + f22, b11, f12 - f22, f21 - f11, b22, f11 + f12, f21 + f22)]


def _strassen_add(init, lhs, rhs_ref):
    order = (0, 1, 3, 4, 2, 6, 5)
    signs = ((1, 0, 0, 1, -1, 0, 1), (0, 0, 1, 0, 1, 0, 0),
             (0, 1, 0, 1, 0, 0, 0), (1, -1, 1, 0, 0, 1, 0))
    prods = {j: _mm(lhs[j], pltpu.bitcast(rhs_ref[j], _BF)) for j in order}
    out = []
    for c, sign in zip(init, signs):
        for j in order:
            if sign[j]:
                c = c + prods[j] if sign[j] > 0 else c - prods[j]
        out.append(c)
    return out


def _silu(g):
    half = 0.5 * g
    return half + half * jnp.tanh(half)


def _after(value, zero):
    return pltpu.bitcast(pltpu.bitcast(value, _U32) | zero, _BF)


def _kernel(x_hbm, wqkv_hbm, wo_hbm, wg_hbm, wu_hbm, wd_hbm, out_hbm,
            x_v, wo_v, wos_v, k_v, kb_v, qf_v, q_v, v_v, y_v, s_v, pos_s,
            x_sem, w_sem, o_sem):
    S, D = x_hbm.shape
    F = wg_hbm.shape[1]
    Dh = D // _H
    G = 8 * Dh
    n_items = S // _W * _H
    n_steps = S // _C
    n_x = len(_X_ROWS) - 1

    def projections(wqkv_v, wt_v, wg_v, wu_v, wd_v, xn_v, kf_v, kp_v, wgs_v, wus_v, wds_v):
        def x_copy(i):
            rows = pl.ds(_X_ROWS[i], _X_ROWS[i + 1] - _X_ROWS[i])
            return pltpu.make_async_copy(x_hbm.at[rows], x_v.at[rows], x_sem.at[i])

        wq_copy, wk_copy, wv_copy = (
            pltpu.make_async_copy(wqkv_hbm.at[:, pl.ds(j * D, D)], wqkv_v.at[j], w_sem.at[j])
            for j in range(3))
        wg_copy, *late_copies = (
            pltpu.make_async_copy(src, dst, w_sem.at[3 + j]) for j, (src, dst) in
            enumerate([(wg_hbm, wg_v), (wu_hbm, wu_v), (wd_hbm, wd_v), (wo_hbm, wo_v)]))

        def layernorm(r0):
            zero = kp_v[pl.ds(pl.multiple_of(pos_s[1], 8), 8), :]
            x = _after(x_v[pl.ds(r0, _TK), :], _cat([zero] * (_TK // 16), 0)).astype(_F32)
            xc = x - jnp.mean(x, axis=-1, keepdims=True)
            var = jnp.mean(xc * xc, axis=-1, keepdims=True)
            xn_v[pl.ds(r0, _TK), :] = (xc * lax.rsqrt(var + _LN_EPS)).astype(_BF)

        def k_projection(r0):
            k = _mm(xn_v[pl.ds(r0, _TK), :], wqkv_v[1]).astype(_BF)
            if r0 < _NV:
                for g in range(_H // 8):
                    kf_v[g, pl.ds(r0, _TK), :] = k.astype(_F32)[:, G * g:G * (g + 1)]
            kp_v[pl.ds(r0 // 2, _TK // 2), :] = pltpu.bitcast(k, _U32)

        x_copy(0).start()
        wk_copy.start()
        for j, pos in enumerate((2 * S, S // 2, n_items, _H)):
            pos_s[j] = pos
        kp_v[pl.ds(S // 2, 8), :] = jnp.zeros((8, D), _U32)
        q_v[n_items, pl.ds(0, 8), pl.ds(0, 128)] = jnp.zeros((8, 128), _U32)
        v_v[_H, pl.ds(0, 8), pl.ds(0, 128)] = jnp.zeros((8, 128), _F32)
        s_v[pl.ds(S - _LAG * _C, S + _LAG * _C), :] = jnp.zeros((S + _LAG * _C, _W), _F32)
        x_copy(0).wait()
        x_copy(1).start()
        layernorm(0)
        wk_copy.wait()
        for r0 in range(0, S, _TK):
            if r0 + _TK in _X_ROWS[:-1]:
                j = _X_ROWS.index(r0 + _TK)
                x_copy(j).wait()
                if j + 1 < n_x:
                    x_copy(j + 1).start()
                if j + 2 == n_x:
                    for copy in (wq_copy, wv_copy, wg_copy):
                        copy.start()
                if j + 1 == n_x:
                    wq_copy.wait()
                    wv_copy.wait()
                    for copy in late_copies:
                        copy.start()
                    wt_v[pl.ds(0, D), :] = wqkv_v[0].T
                    wt_v[pl.ds(D, D), :] = wqkv_v[2].T
            if r0 + _TK < S:
                layernorm(r0 + _TK)
            k_projection(r0)

        def weight_sums(half, weights, part, zero):
            tiles = [(w_v, ws_v, r, c) for w_v, ws_v in weights
                     for r in range(0, ws_v.shape[1], 16) for c in range(0, ws_v.shape[2], 128)]
            for w_v, ws_v, r, c in tiles[part * len(tiles) // 7:(part + 1) * len(tiles) // 7]:
                r = half * ws_v.shape[1] + r
                top = pl.ds(pl.multiple_of(r, 16), 16)
                bottom = pl.ds(pl.multiple_of(2 * ws_v.shape[1] + r, 16), 16)
                left, right = pl.ds(c, 128), pl.ds(ws_v.shape[2] + c, 128)
                for j, b in enumerate(_strassen_rhs(
                        _after(w_v[top, left], zero), w_v[top, right],
                        w_v[bottom, left], _after(w_v[bottom, right], zero))):
                    ws_v[j, pl.ds(pl.multiple_of(r // 2, 8), 8), left] = pltpu.bitcast(b, _U32)

        def qv_step(i, carry, weights):
            toks = pl.ds(pl.multiple_of(i * _T, _T), _T)
            xn = xn_v[toks, :]
            row = lax.broadcasted_iota(jnp.int32, (8, _T), 0)
            zero = jnp.zeros((8, _T), _U32)
            blocks = [(i * (_T // _W) + b, slice(b * _W, (b + 1) * _W)) for b in range(_T // _W)]
            for g in range(_H // 8):
                qt = _mm_nt(wt_v[pl.ds(g * G, G), :], xn)
                qt = (qt * (Dh ** -0.5 * math.log2(math.e))).astype(_BF)
                for b, cols in blocks:
                    qf_v[b * (_H // 8) + g] = qt[:, cols].astype(_F32)
                qt = pltpu.bitcast(qt, _U32)
                for u in range(8):
                    r0, lo = u * Dh // 2 // 8 * 8, u * Dh // 2 % 8
                    q = _cat([jnp.where(row >= lo, qt[r0:r0 + 8], zero),
                              jnp.where(row < lo + Dh // 2 - 8, qt[r0 + 8:r0 + 16], zero)], 0)
                    for b, cols in blocks:
                        q_v[b * _H + 8 * g + u] = q[:, cols]
                weight_sums(i & 1, weights, 2 * g, q_v[pos_s[2], pl.ds(0, 8), pl.ds(0, 128)])

                vt = _mm_nt(wt_v[pl.ds(D + g * G, G), :], xn).astype(_BF).astype(_F32)
                for u in range(8):
                    r0 = u * Dh // 8 * 8
                    if u % 2 == 0:
                        v = [vt[r0:r0 + 16], jnp.where(row == Dh - 16, 1.0, vt[r0 + 16:r0 + 24])]
                    else:
                        v = [jnp.where(row == 0, 1.0, vt[r0:r0 + 8]), vt[r0 + 8:r0 + 24]]
                    v_v[8 * g + u, :, toks] = _cat(v, 0)
                weight_sums(i & 1, weights, 2 * g + 1,
                            pltpu.bitcast(v_v[pos_s[3], pl.ds(0, 8), pl.ds(0, 128)], _U32))
            return carry

        wg_copy.wait()
        lax.fori_loop(0, 2, functools.partial(qv_step, weights=[(wg_v, wgs_v)]), 0)
        for copy in late_copies:
            copy.wait()
        lax.fori_loop(2, 4, functools.partial(
            qv_step, weights=[(wu_v, wus_v), (wd_v, wds_v), (wo_v, wos_v)]), 0)

        def ffn_step(i, carry):
            rows = pl.ds(pl.multiple_of(i * _T, _T), _T)
            xn = xn_v[rows, :]
            xs = _strassen_lhs(*_quarters(xn.astype(_F32), _T // 2, 256))

            def first_layer(w_v, ws_v):
                rest = _mm(xn[:, 512:], w_v[pl.ds(512, D - 512), :])
                return _strassen_add(_quarters(rest, _T // 2, F // 2), xs, ws_v)

            h = [_silu(g) * u for g, u in zip(first_layer(wg_v, wgs_v), first_layer(wu_v, wus_v))]
            x = x_v[rows, :].astype(_F32)
            y_v[rows, pl.ds(0, 512)] = _blocks(
                *_strassen_add(_quarters(x, _T // 2, 256), _strassen_lhs(*h), wds_v))
            y_v[rows, pl.ds(512, D - 512)] = x[:, 512:] + _mm(
                _blocks(*h).astype(_BF), wd_v[:, pl.ds(512, D - 512)])

            packed_rows = pl.ds(pl.multiple_of(i * (_T // 2), _T // 2), _T // 2)
            k = kp_v[packed_rows, :]
            k = _cat([k, k[:, :128]], 1)
            for pair in range(_H // 2):
                lo = pair * 2 * Dh // 16 * 16
                k_v[pair, packed_rows, :] = k[:, lo:lo + 128]
            for d in range(G):
                kb_v[i * 8 + d // Dh, :, pl.ds(d % Dh * 128, 128)] = jnp.broadcast_to(
                    kf_v[i, pl.ds(0, _NV), pl.ds(d, 1)], (_NV, 128))
            return carry

        lax.fori_loop(0, S // _T, ffn_step, 0)

    def attention(qb_v, o_v):
        n_mxu = (S - _NV) // 2
        bounds = [n_mxu // 16 * c // n_steps * 16 for c in range(n_steps + 1)]
        vpu_tiles = [(r0, t) for r0 in range(0, _NV, 8) for t in range(_W // 128)]

        def update_max(m, s, t0):
            m = list(m)
            for t in range(s.shape[1] // 128):
                part = jnp.max(s[:, t * 128:(t + 1) * 128].reshape(-1, 8, 128), axis=0)
                m[t0 + t] = part if m[t0 + t] is None else jnp.maximum(m[t0 + t], part)
            return m

        def repeat_q(item, u, features):
            for d in features:
                r0, r = divmod(u % 8 * Dh + d, 8)
                q = qf_v[(item & (n_items - 1)) >> 3, pl.ds(8 * r0, 8), :]
                q = jnp.broadcast_to(q[r:r + 1], (8, _W))
                if d == _PACED:
                    s_v[pl.ds(2 * S + u % 2 * 16, 8), :] = q
                else:
                    qb_v[u % 2, d] = q

        def vpu_scores(pos, item, u, r0, t, m):
            lanes = pl.ds(t * 128, 128)
            sums = [None, None]
            for d in range(Dh):
                if d == _PACED:
                    q = s_v[pl.ds(pos + u % 2 * 16, 8), lanes]
                else:
                    q = qb_v[u % 2, d, :, lanes]
                term = kb_v[item & (_H - 1), pl.ds(r0, 8), pl.ds(d * 128, 128)] * q
                sums[d % 2] = term if sums[d % 2] is None else sums[d % 2] + term
            s = sums[0] + sums[1]
            s_v[pl.ds(u % 2 * S + r0, 8), lanes] = s
            return update_max(m, s, t)

        def scores(pos, item, u, c, m):
            above = u % 8 * Dh // 16 - u % 8 // 2 * 2 * Dh // 16
            zero = jnp.zeros((8, _W), _U32)
            q = pltpu.bitcast(_cat([zero] * above + [q_v[item]] + [zero] * (6 - above), 0), _BF)
            lo, hi = bounds[c], bounds[c + 1]
            halves = []
            for r0 in (_NV + lo, _NV + n_mxu + lo):
                k = k_v[(item & (_H - 1)) >> 1, pl.ds(r0 // 2, (hi - lo) // 2), :]
                halves.append((r0, _mm(pltpu.bitcast(k, _BF), q)))
            stops = [(e + 1) * n_mxu / len(vpu_tiles) - lo for e in range(len(vpu_tiles))]
            stops = [(round(at / 8) * 8, tile)
                     for at, tile in zip(stops, vpu_tiles) if 0 < at <= hi - lo]
            done = 0
            for upto, tile in stops + [(hi - lo, None)]:
                if upto > done:
                    for r0, s in halves:
                        s_v[pl.ds(u % 2 * S + r0 + done, upto - done), :] = s[done:upto]
                    done = upto
                if tile is not None:
                    m = vpu_scores(pos, item, u, *tile, m)
            for _, s in halves:
                m = update_max(m, s, 0)
            return m

        def weighted_values(item, u, c, m, acc):
            p = jnp.exp2(s_v[pl.ds(u % 2 * S + c * _C, _C), :] - m).astype(_BF)
            o = _mm(v_v[item & (_H - 1), :, pl.ds(c * _C, _C)], p)
            return o if c == 0 else acc + o

        def attention_step(i, carry):
            acc, m2, m1 = carry
            pos = pl.multiple_of(pos_s[0], 16)
            for u in range(_UNROLL):
                item = i * _UNROLL + u
                m = [None] * (_W // 128)
                for c in range(n_steps):
                    m = scores(pos, item, u, c, m)
                    if c < _LAG:
                        acc = weighted_values(item - 2, u - 2, n_steps - _LAG + c, m2, acc)
                    else:
                        acc = weighted_values(item - 1, u - 1, c - _LAG, m1, acc)
                    if c == _LAG - 1:
                        o_v[item] = acc
                    repeat_q(item + 1, u + 1, range(c * Dh // n_steps, (c + 1) * Dh // n_steps))
                m2, m1 = m1, jnp.max(_cat(m, 1), axis=0, keepdims=True)
            return acc, m2, m1

        repeat_q(0, 0, range(Dh))
        acc, m2, m1 = lax.fori_loop(
            0, n_items // _UNROLL, attention_step,
            (jnp.zeros((24, _W), _F32), jnp.zeros((1, _W), _F32), jnp.zeros((1, _W), _F32)))

        def out_copy(b):
            rows = pl.ds(b * _W, _W)
            return pltpu.make_async_copy(x_v.at[rows], out_hbm.at[rows], o_sem.at[b])

        def merged_heads(b, t):
            row = lax.broadcasted_iota(jnp.int32, (8, 128), 0)
            parts = []
            for h in range(0, _H, 2):
                even = o_v[b * _H + h + 2, :, pl.ds(t * 128, 128)]
                odd = o_v[b * _H + h + 3, :, pl.ds(t * 128, 128)]
                even = even * (1.0 / even[Dh:Dh + 1])
                odd = odd * (1.0 / odd[0:1])
                parts += [even[:16], jnp.where(row < Dh - 16, even[16:], odd[:8]), odd[8:]]
            return _cat(parts, 0).T

        for c in range(n_steps - _LAG, n_steps):
            acc = weighted_values(n_items - 2, 0, c, m2, acc)
        o_v[n_items] = acc
        for b in range(S // _W):
            rows = pl.ds(b * _W, _W)
            o = _cat([merged_heads(b, t) for t in range(_W // 128)], 0)
            y = y_v[rows, :]
            right = y[:, 512:] + _mm(o.astype(_BF), wo_v[:, pl.ds(512, D - 512)])
            left = y[:, :512] + _mm(
                o.astype(_BF)[:, 512:], wo_v[pl.ds(512, D - 512), pl.ds(0, 512)])
            left = _strassen_add(_quarters(left, _W // 2, 256),
                                 _strassen_lhs(*_quarters(o, _W // 2, 256)), wos_v)
            x_v[rows, :] = _cat([_blocks(*left), right], 1).astype(_BF)
            out_copy(b).start()
            for c in range(2 * b, min(n_steps, 2 * b + 2)):
                acc = weighted_values(n_items - 1, 1, c, m1, acc)
                if c == n_steps - 1:
                    o_v[n_items + 1] = acc
        for b in range(S // _W):
            out_copy(b).wait()

    pl.run_scoped(
        projections,
        pltpu.VMEM((3, D, D), _BF),
        pltpu.VMEM((2 * D, D), _BF),
        pltpu.VMEM((D, F), _BF),
        pltpu.VMEM((D, F), _BF),
        pltpu.VMEM((F, D), _BF),
        pltpu.VMEM((S, D), _BF),
        pltpu.VMEM((_H // 8, pl.cdiv(_NV, _TK) * _TK, G), _F32),
        pltpu.VMEM((S // 2 + 8, D), _U32),
        pltpu.VMEM((7, 128, F // 2), _U32),
        pltpu.VMEM((7, 128, F // 2), _U32),
        pltpu.VMEM((7, F // 4, 256), _U32))
    pl.run_scoped(
        attention,
        pltpu.VMEM((2, Dh, 8, _W), _F32),
        pltpu.VMEM((n_items + 2, 24, _W), _F32))


@jax.jit
def pallas_parallel_sum__mha_block__swiglu_ffn__prompt_kernel(
    A_x: jax.Array,
    A_wqkv: jax.Array,
    A_wo: jax.Array,
    B_x: jax.Array,
    B_w_gate: jax.Array,
    B_w_up: jax.Array,
    B_w_down: jax.Array,
):
    del B_x
    B, S, D = A_x.shape
    assert (B, S, D, B_w_gate.shape[1]) == (1, 2048, 640, 1536)
    Dh = D // _H
    n_items = S // _W * _H
    in_hbm = pl.BlockSpec(memory_space=pl.ANY)
    out = pl.pallas_call(
        _kernel,
        out_shape=jax.ShapeDtypeStruct((S, D), A_x.dtype),
        in_specs=[in_hbm] * 6,
        out_specs=in_hbm,
        scratch_shapes=[
            pltpu.VMEM((S, D), _BF),
            pltpu.VMEM((D, D), _BF),
            pltpu.VMEM((7, 128, 256), _U32),
            pltpu.VMEM((_H // 2, S // 2, 128), _U32),
            pltpu.VMEM((_H, _NV, Dh * 128), _F32),
            pltpu.VMEM((n_items // 8, 8 * Dh, _W), _F32),
            pltpu.VMEM((n_items + 1, 16, _W), _U32),
            pltpu.VMEM((_H + 1, 24, S), _F32),
            pltpu.VMEM((S, D), _F32),
            pltpu.VMEM((2 * S + 32, _W), _F32),
            pltpu.SMEM((4,), jnp.int32),
            pltpu.SemaphoreType.DMA((len(_X_ROWS) - 1,)),
            pltpu.SemaphoreType.DMA((7,)),
            pltpu.SemaphoreType.DMA((S // _W,)),
        ],
        compiler_params=pltpu.CompilerParams(vmem_limit_bytes=124 * 2**20),
    )(A_x.reshape(S, D), A_wqkv, A_wo, B_w_gate, B_w_up, B_w_down)
    return out.reshape(B, S, D)
```
